```python
import jax
import jax.numpy as jnp

def _softmax(x, axis=-1):
    return jax.nn.softmax(x, axis=axis)
def _gelu(x):
    return jax.nn.gelu(x, approximate=True)
def _silu(x):
    return jax.nn.silu(x)
def _sigmoid(x):
    return jax.nn.sigmoid(x)
def _layernorm(x, axis=-1, eps=1e-5):
    m = jnp.mean(x, axis=axis, keepdims=True)
    v = jnp.var(x, axis=axis, keepdims=True)
    return (x - m) / jnp.sqrt(v + eps)
def _scatter_add(tgt, idx, src, axis=0):
    return tgt.at[idx].add(src)
def _segment_sum(src, seg, n):
    return jax.ops.segment_sum(src, seg, n)
class _Rng:
    def __init__(self, key):
        self._k = key
    def _next(self):
        self._k, sub = jax.random.split(self._k)
        return sub
    def normal(self, shape):
        return jax.random.normal(self._next(), shape, dtype=jnp.bfloat16)
    def randint(self, lo, hi, shape):
        return jax.random.randint(self._next(), shape, lo, hi, dtype=jnp.int32)
    def uniform(self, shape, lo=0.0, hi=1.0):
        return jax.random.uniform(self._next(), shape, jnp.bfloat16, lo, hi)
    def permutation(self, n):
        return jax.random.permutation(self._next(), n)


kernel_name = 'sequential_preLN__mha_block_cached__moe_arch_mod__decode'

def setup_inputs():
    _rng = _Rng(jax.random.key(int.from_bytes(__import__("os").urandom(4), "little")))
    _w = (lambda a: (lambda t: t.astype(jnp.bfloat16) if jnp.issubdtype(t.dtype, jnp.floating) else t)(jnp.asarray(a)))
    def _A_setup():
        B, Sq, D = 4, 1, 640
        H, Sk, Dh = 32, 8192, 192
        return {
            "x": _w((lambda *s: _rng.normal(s) * 0.05)(B, Sq, D)),
            "k_cache": _w((lambda *s: _rng.normal(s) * 0.05)(B, H, Sk, Dh)),
            "v_cache": _w((lambda *s: _rng.normal(s) * 0.05)(B, H, Sk, Dh)),
            "wq": _w((lambda *s: _rng.normal(s) * 0.05)(D, H * Dh) * (D ** -0.5)),
            "wo": _w((lambda *s: _rng.normal(s) * 0.05)(H * Dh, D) * ((H * Dh) ** -0.5)),
        }
    _A_in = _A_setup()

    def _B_setup():
        B, S, D, F, C = 4, 1, 640, 1536, 1
        return {
            "x": _w((lambda *s: _rng.normal(s) * 0.05)(B, S, D)),
            "w_r": _w((lambda *s: _rng.normal(s) * 0.05)(D)),
            "w_gate": _w((lambda *s: _rng.normal(s) * 0.05)(D, F)),
            "w_up": _w((lambda *s: _rng.normal(s) * 0.05)(D, F)),
            "w_down": _w((lambda *s: _rng.normal(s) * 0.05)(F, D)),
        }
    _B_in = _B_setup()

    return {
        "A_x": _A_in["x"],
        "A_k_cache": _A_in["k_cache"],
        "A_v_cache": _A_in["v_cache"],
        "A_wq": _A_in["wq"],
        "A_wo": _A_in["wo"],
        "B_x": _B_in["x"],
        "B_w_r": _B_in["w_r"],
        "B_w_gate": _B_in["w_gate"],
        "B_w_up": _B_in["w_up"],
        "B_w_down": _B_in["w_down"],
    }

def reference(A_x, A_k_cache, A_v_cache, A_wq, A_wo, B_x, B_w_r, B_w_gate, B_w_up, B_w_down):
    def _A_ref(x, k_cache, v_cache, wq, wo):
        B, Sq, D = x.shape
        H, Dh = 32, 192
        q = (lambda x, *d: x.transpose(*d))((x @ wq).reshape(B, Sq, H, Dh), 0, 2, 1, 3)
        scores = jnp.einsum("bhqd,bhkd->bhqk", q, k_cache) * (Dh ** -0.5)
        p = _softmax(scores, axis=-1)
        o = jnp.einsum("bhqk,bhkd->bhqd", p, v_cache)
        return (lambda x, *d: x.transpose(*d))(o, 0, 2, 1, 3).reshape(B, Sq, H * Dh) @ wo

    def _B_ref(x, w_r, w_gate, w_up, w_down):
        B, S, D = x.shape
        C = 1
        r = x @ w_r
        idx = jnp.argsort(-r, axis=-1)[:, :C]
        idx_e = jnp.repeat(idx.reshape(B, C, 1), D, axis=2)
        x_sel = jnp.take_along_axis(x, idx_e, axis=1)
        g = _silu(x_sel @ w_gate)
        u = x_sel @ w_up
        y = (g * u) @ w_down
        r_sel = _sigmoid(jnp.take_along_axis(r, idx, axis=1))
        y = y * r_sel.reshape(B, C, 1)
        b_off = (jnp.arange(B) * S).reshape(B, 1)
        flat_idx = (idx + b_off).reshape(B * C)
        zero = (x * 0.0).reshape(B * S, D)
        upd = _scatter_add(zero, flat_idx, y.reshape(B * C, D), axis=0)
        return x + upd.reshape(B, S, D)

    x = A_x
    h = x + _A_ref(_layernorm(x, axis=-1), A_k_cache, A_v_cache, A_wq, A_wo)
    h2 = h + _B_ref(_layernorm(h, axis=-1), B_w_r, B_w_gate, B_w_up, B_w_down)
    return h2
```

```python
import functools

import jax
import jax.numpy as jnp
import jax.experimental.pallas as pl
import jax.experimental.pallas.tpu as pltpu

_LN_EPS = 1e-5
_NB = 4
_WD_CHUNKS = 4


def _layernorm(x):
    m = jnp.mean(x, axis=-1, keepdims=True)
    d = x - m
    v = jnp.mean(d * d, axis=-1, keepdims=True)
    return d / jnp.sqrt(v + _LN_EPS)


def _pad_rows(a, rows):
    return jnp.concatenate([a, jnp.zeros((rows - a.shape[0], a.shape[1]), a.dtype)], axis=0)


def _kernel(x_hbm, kt_hbm, vt_hbm, wq_hbm, wo_hbm, wr_ref, wg_hbm, wu_hbm, wd_hbm,
            out_hbm,
            kv_buf, x_buf, wq_buf, wo_buf, wg_buf, wu_buf, wd_buf,
            q_scr, oh_scr, acc_scr, out_buf,
            kv_sems, w_sems, wd_sems,
            *, B, H, S, Dh, D, F):
    n_steps = B * H
    n_items = 2 * n_steps
    scale = Dh ** -0.5
    bf16 = jnp.bfloat16
    f32 = jnp.float32

    def slab_index(step):
        return step % B, step // B

    def k_copy(step, slot):
        b, h = slab_index(step)
        return pltpu.make_async_copy(kt_hbm.at[b, h], kv_buf.at[slot], kv_sems.at[slot])

    def v_copy(step, slot):
        b, h = slab_index(step)
        return pltpu.make_async_copy(vt_hbm.at[b, h], kv_buf.at[slot], kv_sems.at[slot])

    x_copy = pltpu.make_async_copy(x_hbm, x_buf, w_sems.at[0])
    wq_copy = pltpu.make_async_copy(wq_hbm, wq_buf, w_sems.at[1])
    wo_copy = pltpu.make_async_copy(wo_hbm, wo_buf, w_sems.at[2])
    wg_copy = pltpu.make_async_copy(wg_hbm, wg_buf, w_sems.at[3])
    wu_copy = pltpu.make_async_copy(wu_hbm, wu_buf, w_sems.at[4])
    out_copy = pltpu.make_async_copy(out_buf, out_hbm, w_sems.at[5])
    fc = F // _WD_CHUNKS

    def wd_copy(c):
        return pltpu.make_async_copy(
            wd_hbm.at[pl.ds(c * fc, fc)], wd_buf.at[pl.ds(c * fc, fc)], wd_sems.at[c])

    x_copy.start()
    wq_copy.start()
    pairs_in_flight = _NB // 2
    for s in range(pairs_in_flight):
        k_copy(s, 2 * s).start()
        v_copy(s, 2 * s + 1).start()
    wo_copy.start()

    x_copy.wait()
    x32 = x_buf[...].astype(f32)
    xn = _pad_rows(_layernorm(x32), 8).astype(bf16)
    wq_copy.wait()
    q_all = jnp.dot(xn, wq_buf[...], preferred_element_type=f32)
    for h in range(H):
        q_scr[h] = q_all[:, h * Dh:(h + 1) * Dh]
    acc_scr[...] = jnp.zeros_like(acc_scr)
    oh_scr[...] = jnp.zeros_like(oh_scr)

    row = jax.lax.broadcasted_iota(jnp.int32, (8, Dh), 0)

    def step_body(step, carry):
        b, h = slab_index(step)
        kslot = (2 * step) % _NB
        vslot = kslot + 1
        nxt = step + pairs_in_flight

        q = q_scr[h].astype(bf16)
        k_copy(step, kslot).wait()
        s = jnp.dot(q, kv_buf[kslot], preferred_element_type=f32)

        @pl.when(nxt < n_steps)
        def _():
            k_copy(nxt, kslot).start()

        m = jnp.max(s, axis=1, keepdims=True)
        p = jnp.exp((s - m) * scale)
        l = jnp.sum(p, axis=1, keepdims=True)
        v_copy(step, vslot).wait()
        o = jax.lax.dot_general(p.astype(bf16), kv_buf[vslot], (((1,), (1,)), ((), ())),
                                preferred_element_type=f32)

        @pl.when(nxt < n_steps)
        def _():
            v_copy(nxt, vslot).start()

        @pl.when(nxt == n_steps - 1)
        def _():
            wg_copy.start()
            wu_copy.start()
            for c in range(_WD_CHUNKS):
                wd_copy(c).start()

        oh_scr[...] = jnp.where(row == b, o / l, oh_scr[...])

        @pl.when(step == B - 1)
        def _():
            wo_copy.wait()

        @pl.when(b == B - 1)
        def _():
            off = pl.multiple_of(h * Dh, Dh)
            acc_scr[...] += jnp.dot(oh_scr[...].astype(bf16), wo_buf[pl.ds(off, Dh), :],
                                    preferred_element_type=f32)

        return carry

    jax.lax.fori_loop(0, n_steps, step_body, 0)

    hres = x32 + acc_scr[0:B, :]
    hn = _layernorm(hres)
    hn8 = _pad_rows(hn, 8).astype(bf16)
    r = jnp.sum(hn * wr_ref[...].astype(f32), axis=-1, keepdims=True)
    gate = jax.nn.sigmoid(r)
    wg_copy.wait()
    g = jnp.dot(hn8, wg_buf[...], preferred_element_type=f32)
    g = g * jax.nn.sigmoid(g)
    wu_copy.wait()
    u = jnp.dot(hn8, wu_buf[...], preferred_element_type=f32)
    act = (g * u).astype(bf16)
    y = jnp.zeros((8, D), f32)
    for c in range(_WD_CHUNKS):
        wd_copy(c).wait()
        y = y + jnp.dot(act[:, c * fc:(c + 1) * fc], wd_buf[pl.ds(c * fc, fc), :],
                        preferred_element_type=f32)
    out_buf[...] = (hn + y[0:B, :] * gate).astype(out_buf.dtype)
    out_copy.start()
    out_copy.wait()


@jax.jit
def pallas_sequential_preLN__mha_block_cached__moe_arch_mod__decode_kernel(
    A_x: jax.Array,
    A_k_cache: jax.Array,
    A_v_cache: jax.Array,
    A_wq: jax.Array,
    A_wo: jax.Array,
    B_x: jax.Array,
    B_w_r: jax.Array,
    B_w_gate: jax.Array,
    B_w_up: jax.Array,
    B_w_down: jax.Array,
):
    B, Sq, D = A_x.shape
    _, H, S, Dh = A_k_cache.shape
    F = B_w_gate.shape[1]
    assert Sq == 1
    x = A_x.reshape(B, D)
    kt = A_k_cache.transpose(0, 1, 3, 2)
    vt = A_v_cache.transpose(0, 1, 3, 2)
    wr = B_w_r.reshape(1, D)
    any_spec = pl.BlockSpec(memory_space=pl.ANY)
    vmem_spec = pl.BlockSpec(memory_space=pltpu.VMEM)
    bf16 = jnp.bfloat16
    out = pl.pallas_call(
        functools.partial(_kernel, B=B, H=H, S=S, Dh=Dh, D=D, F=F),
        out_shape=jax.ShapeDtypeStruct((B, D), A_x.dtype),
        in_specs=[any_spec, any_spec, any_spec, any_spec, any_spec, vmem_spec,
                  any_spec, any_spec, any_spec],
        out_specs=any_spec,
        scratch_shapes=[
            pltpu.VMEM((_NB, Dh, S), bf16),
            pltpu.VMEM((B, D), bf16),
            pltpu.VMEM((D, H * Dh), bf16),
            pltpu.VMEM((H * Dh, D), bf16),
            pltpu.VMEM((D, F), bf16),
            pltpu.VMEM((D, F), bf16),
            pltpu.VMEM((F, D), bf16),
            pltpu.VMEM((H, 8, Dh), jnp.float32),
            pltpu.VMEM((8, Dh), jnp.float32),
            pltpu.VMEM((8, D), jnp.float32),
            pltpu.VMEM((B, D), bf16),
            pltpu.SemaphoreType.DMA((_NB,)),
            pltpu.SemaphoreType.DMA((6,)),
            pltpu.SemaphoreType.DMA((_WD_CHUNKS,)),
        ],
        compiler_params=pltpu.CompilerParams(vmem_limit_bytes=64 * 1024 * 1024),
    )(x, kt, vt, A_wq, A_wo, wr, B_w_gate, B_w_up, B_w_down)
    return out.reshape(B, Sq, D)
```

```python
import functools

import jax
import jax.numpy as jnp
import jax.experimental.pallas as pl
import jax.experimental.pallas.tpu as pltpu

_LN_EPS = 1e-5
_NB = 4
_STRIP = 128
_WD_CHUNKS = 4


def _layernorm(x):
    m = jnp.mean(x, axis=-1, keepdims=True)
    d = x - m
    v = jnp.mean(d * d, axis=-1, keepdims=True)
    return d / jnp.sqrt(v + _LN_EPS)


def _pad_rows(a, rows):
    return jnp.concatenate([a, jnp.zeros((rows - a.shape[0], a.shape[1]), a.dtype)], axis=0)


def _kernel(x_hbm, kt_hbm, vt_hbm, wq_hbm, wo_hbm, wr_ref, wg_hbm, wu_hbm, wd_hbm,
            out_hbm,
            kv_buf, x_buf, wq_buf, wo_buf, wg_buf, wu_buf, wd_buf,
            q_scr, oh_scr, acc_scr, out_buf,
            kv_sems, w_sems, wd_sems,
            *, B, H, S, Dh, D, F):
    n_steps = B * H
    n_items = 2 * n_steps
    scale = Dh ** -0.5
    bf16 = jnp.bfloat16
    f32 = jnp.float32

    def slab_index(step):
        return step % B, step // B

    n_strips = S // _STRIP

    def issue_slab(src_hbm, step, slot):
        b, h = slab_index(step)
        for c in range(n_strips):
            cols = pl.ds(c * _STRIP, _STRIP)
            pltpu.make_async_copy(src_hbm.at[b, h, :, cols], kv_buf.at[slot, :, cols],
                                  kv_sems.at[slot]).start(priority=c % 2)

    def wait_slab(slot):
        pltpu.make_async_copy(kv_buf.at[slot], kv_buf.at[slot], kv_sems.at[slot]).wait()

    x_copy = pltpu.make_async_copy(x_hbm, x_buf, w_sems.at[0])
    wq_copy = pltpu.make_async_copy(wq_hbm, wq_buf, w_sems.at[1])
    wo_copy = pltpu.make_async_copy(wo_hbm, wo_buf, w_sems.at[2])
    wg_copy = pltpu.make_async_copy(wg_hbm, wg_buf, w_sems.at[3])
    wu_copy = pltpu.make_async_copy(wu_hbm, wu_buf, w_sems.at[4])
    out_copy = pltpu.make_async_copy(out_buf, out_hbm, w_sems.at[5])
    fc = F // _WD_CHUNKS

    def wd_copy(c):
        return pltpu.make_async_copy(
            wd_hbm.at[pl.ds(c * fc, fc)], wd_buf.at[pl.ds(c * fc, fc)], wd_sems.at[c])

    x_copy.start()
    wq_copy.start()
    pairs_in_flight = _NB // 2
    for s in range(pairs_in_flight):
        issue_slab(kt_hbm, s, 2 * s)
        issue_slab(vt_hbm, s, 2 * s + 1)
    wo_copy.start()

    x_copy.wait()
    x32 = x_buf[...].astype(f32)
    xn = _pad_rows(_layernorm(x32), 8).astype(bf16)
    wq_copy.wait()
    q_all = jnp.dot(xn, wq_buf[...], preferred_element_type=f32)
    for h in range(H):
        q_scr[h] = q_all[:, h * Dh:(h + 1) * Dh]
    acc_scr[...] = jnp.zeros_like(acc_scr)
    oh_scr[...] = jnp.zeros_like(oh_scr)

    row = jax.lax.broadcasted_iota(jnp.int32, (8, Dh), 0)

    def step_body(step, carry):
        b, h = slab_index(step)
        kslot = (2 * step) % _NB
        vslot = kslot + 1
        nxt = step + pairs_in_flight

        q = q_scr[h].astype(bf16)
        wait_slab(kslot)
        s = jnp.dot(q, kv_buf[kslot], preferred_element_type=f32)

        @pl.when(nxt < n_steps)
        def _():
            issue_slab(kt_hbm, nxt, kslot)

        m = jnp.max(s, axis=1, keepdims=True)
        p = jnp.exp((s - m) * scale)
        l = jnp.sum(p, axis=1, keepdims=True)
        wait_slab(vslot)
        o = jax.lax.dot_general(p.astype(bf16), kv_buf[vslot], (((1,), (1,)), ((), ())),
                                preferred_element_type=f32)

        @pl.when(nxt < n_steps)
        def _():
            issue_slab(vt_hbm, nxt, vslot)

        @pl.when(nxt == n_steps - 1)
        def _():
            wg_copy.start()
            wu_copy.start()
            for c in range(_WD_CHUNKS):
                wd_copy(c).start()

        oh_scr[...] = jnp.where(row == b, o / l, oh_scr[...])

        @pl.when(step == B - 1)
        def _():
            wo_copy.wait()

        @pl.when(b == B - 1)
        def _():
            off = pl.multiple_of(h * Dh, Dh)
            acc_scr[...] += jnp.dot(oh_scr[...].astype(bf16), wo_buf[pl.ds(off, Dh), :],
                                    preferred_element_type=f32)

        return carry

    jax.lax.fori_loop(0, n_steps, step_body, 0)

    hres = x32 + acc_scr[0:B, :]
    hn = _layernorm(hres)
    hn8 = _pad_rows(hn, 8).astype(bf16)
    r = jnp.sum(hn * wr_ref[...].astype(f32), axis=-1, keepdims=True)
    gate = jax.nn.sigmoid(r)
    wg_copy.wait()
    g = jnp.dot(hn8, wg_buf[...], preferred_element_type=f32)
    g = g * jax.nn.sigmoid(g)
    wu_copy.wait()
    u = jnp.dot(hn8, wu_buf[...], preferred_element_type=f32)
    act = (g * u).astype(bf16)
    y = jnp.zeros((8, D), f32)
    for c in range(_WD_CHUNKS):
        wd_copy(c).wait()
        y = y + jnp.dot(act[:, c * fc:(c + 1) * fc], wd_buf[pl.ds(c * fc, fc), :],
                        preferred_element_type=f32)
    out_buf[...] = (hres + (hn + y[0:B, :] * gate)).astype(out_buf.dtype)
    out_copy.start()
    out_copy.wait()


@jax.jit
def pallas_sequential_preLN__mha_block_cached__moe_arch_mod__decode_kernel(
    A_x: jax.Array,
    A_k_cache: jax.Array,
    A_v_cache: jax.Array,
    A_wq: jax.Array,
    A_wo: jax.Array,
    B_x: jax.Array,
    B_w_r: jax.Array,
    B_w_gate: jax.Array,
    B_w_up: jax.Array,
    B_w_down: jax.Array,
):
    B, Sq, D = A_x.shape
    _, H, S, Dh = A_k_cache.shape
    F = B_w_gate.shape[1]
    assert Sq == 1
    x = A_x.reshape(B, D)
    kt = A_k_cache.transpose(0, 1, 3, 2)
    vt = A_v_cache.transpose(0, 1, 3, 2)
    wr = B_w_r.reshape(1, D)
    any_spec = pl.BlockSpec(memory_space=pl.ANY)
    vmem_spec = pl.BlockSpec(memory_space=pltpu.VMEM)
    bf16 = jnp.bfloat16
    out = pl.pallas_call(
        functools.partial(_kernel, B=B, H=H, S=S, Dh=Dh, D=D, F=F),
        out_shape=jax.ShapeDtypeStruct((B, D), A_x.dtype),
        in_specs=[any_spec, any_spec, any_spec, any_spec, any_spec, vmem_spec,
                  any_spec, any_spec, any_spec],
        out_specs=any_spec,
        scratch_shapes=[
            pltpu.VMEM((_NB, Dh, S), bf16),
            pltpu.VMEM((B, D), bf16),
            pltpu.VMEM((D, H * Dh), bf16),
            pltpu.VMEM((H * Dh, D), bf16),
            pltpu.VMEM((D, F), bf16),
            pltpu.VMEM((D, F), bf16),
            pltpu.VMEM((F, D), bf16),
            pltpu.VMEM((H, 8, Dh), jnp.float32),
            pltpu.VMEM((8, Dh), jnp.float32),
            pltpu.VMEM((8, D), jnp.float32),
            pltpu.VMEM((B, D), bf16),
            pltpu.SemaphoreType.DMA((_NB,)),
            pltpu.SemaphoreType.DMA((6,)),
            pltpu.SemaphoreType.DMA((_WD_CHUNKS,)),
        ],
        compiler_params=pltpu.CompilerParams(vmem_limit_bytes=64 * 1024 * 1024),
    )(x, kt, vt, A_wq, A_wo, wr, B_w_gate, B_w_up, B_w_down)
    return out.reshape(B, Sq, D)
```

```python
import contextlib
import functools

import jax
import jax.numpy as jnp
import jax.experimental.pallas as pl
import jax.experimental.pallas.tpu as pltpu

_LN_EPS = 1e-5
_NB = 3
_HG = 2
_STRIP = 128
_WD_CHUNKS = 4
_WQ_RB = 320
_WO_WIN = (48, 640)
_WG_WIN = (320, 128)
_WD_WIN = (48, 640)
_UNROLL = 2
_SCOPES = False
_NOBOUNDS = True
_DBG_STEPS = None


def _scope(name):
    return jax.named_scope(name) if _SCOPES else contextlib.nullcontext()


def _layernorm(x):
    m = jnp.mean(x, axis=-1, keepdims=True)
    d = x - m
    v = jnp.mean(d * d, axis=-1, keepdims=True)
    return d / jnp.sqrt(v + _LN_EPS)


def _pad_rows(a, rows):
    return jnp.concatenate([a, jnp.zeros((rows - a.shape[0], a.shape[1]), a.dtype)], axis=0)


def _issue_windows(src, dst, sem, row_block, col_block):
    rows, cols = src.shape

    def start(r, c, priority):
        win = (pl.ds(r, row_block), pl.ds(c, col_block))
        pltpu.make_async_copy(src.at[win], dst.at[win], sem).start(priority=priority)

    if col_block == cols:
        n = rows // row_block
        assert n % (2 * _UNROLL) == 0

        def body(i, carry):
            for u in range(2 * _UNROLL):
                r = pl.multiple_of((2 * _UNROLL * i + u) * row_block, row_block)
                start(r, 0, u % 2)
            return carry

        jax.lax.fori_loop(0, n // (2 * _UNROLL), body, 0)
    else:
        n = cols // col_block
        assert n % (2 * _UNROLL) == 0
        for r in range(0, rows, row_block):
            def body(i, carry, r=r):
                for u in range(2 * _UNROLL):
                    c = pl.multiple_of((2 * _UNROLL * i + u) * col_block, col_block)
                    start(r, c, u % 2)
                return carry

            jax.lax.fori_loop(0, n // (2 * _UNROLL), body, 0)


def _wait_all(dst, sem):
    pltpu.make_async_copy(dst, dst, sem).wait()


def _kernel(x_hbm, kt_hbm, vt_hbm, wq_hbm, wo_hbm, wr_ref, wg_hbm, wu_hbm, wd_hbm,
            out_hbm,
            kv_buf, x_buf, wq_buf, wo_buf, wg_buf, wu_buf, wd_buf,
            q_scr, oh_scr, acc_scr, out_buf,
            kv_sems, w_sems, wd_sems,
            *, B, G, S, Dh, D, F):
    GD = _HG * Dh
    n_steps = _DBG_STEPS or B * G
    assert _NB == 3
    scale = Dh ** -0.5
    bf16 = jnp.bfloat16
    f32 = jnp.float32

    def slab_index(step):
        return step % B, step // B

    def issue_slab(src_hbm, step, slot):
        b, g = slab_index(step)
        _issue_windows(src_hbm.at[b, g], kv_buf.at[slot], kv_sems.at[slot], GD, _STRIP)

    def wait_slab(slot):
        _wait_all(kv_buf.at[slot], kv_sems.at[slot])

    x_copy = pltpu.make_async_copy(x_hbm, x_buf, w_sems.at[0])
    out_copy = pltpu.make_async_copy(out_buf, out_hbm, w_sems.at[5])
    fc = F // _WD_CHUNKS

    with _scope("p_issue"):
        x_copy.start()
        _issue_windows(wq_hbm, wq_buf, w_sems.at[1], _WQ_RB, _STRIP)
        issue_slab(kt_hbm, 0, 0)
        issue_slab(vt_hbm, 0, 1)

    with _scope("p_ln"):
        x_copy.wait()
        x32 = x_buf[...].astype(f32)
        xn = _pad_rows(_layernorm(x32), 8).astype(bf16)
    with _scope("p_wqwait"):
        _wait_all(wq_buf, w_sems.at[1])
    with _scope("p_qproj"):
        q_all = jnp.dot(xn, wq_buf[...], preferred_element_type=f32)
        for g in range(G):
            q_scr[g] = q_all[:, g * GD:(g + 1) * GD]
        acc_scr[...] = jnp.zeros_like(acc_scr)
        oh_scr[...] = jnp.zeros_like(oh_scr)

    row = jax.lax.broadcasted_iota(jnp.int32, (8, GD), 0)
    lane = jax.lax.broadcasted_iota(jnp.int32, (8, GD), 1)
    diag = jnp.logical_and(lane >= row * Dh, lane < (row + 1) * Dh)

    def step_body(step, carry):
        b, g = slab_index(step)
        kslot = (2 * step) % _NB
        vslot = (2 * step + 1) % _NB
        nslot = (2 * step + 2) % _NB
        last = step == n_steps - 1

        @pl.when(jnp.logical_not(last))
        def _():
            with _scope("issueK"):
                issue_slab(kt_hbm, step + 1, nslot)

        @pl.when(last)
        def _():
            with _scope("issueW"):
                _issue_windows(wg_hbm, wg_buf, w_sems.at[3], *_WG_WIN)
                _issue_windows(wu_hbm, wu_buf, w_sems.at[4], *_WG_WIN)
                for c in range(_WD_CHUNKS):
                    rows = pl.ds(c * fc, fc)
                    _issue_windows(wd_hbm.at[rows], wd_buf.at[rows], wd_sems.at[c], *_WD_WIN)

        qb = jnp.sum(jnp.where(row == b, q_scr[g], 0.0), axis=0, keepdims=True)
        q = jnp.where(diag, qb, 0.0).astype(bf16)
        with _scope("waitK"):
            wait_slab(kslot)
        with _scope("qk"):
            s = jnp.dot(q, kv_buf[kslot], preferred_element_type=f32)

        @pl.when(jnp.logical_not(last))
        def _():
            with _scope("issueV"):
                issue_slab(vt_hbm, step + 1, kslot)

        @pl.when(step == 0)
        def _():
            with _scope("issueWo"):
                _issue_windows(wo_hbm, wo_buf, w_sems.at[2], *_WO_WIN)

        m = jnp.max(s, axis=1, keepdims=True)
        p = jnp.exp((s - m) * scale)
        l = jnp.sum(p, axis=1, keepdims=True)
        with _scope("waitV"):
            wait_slab(vslot)
        with _scope("pv"):
            o = jax.lax.dot_general(p.astype(bf16), kv_buf[vslot], (((1,), (1,)), ((), ())),
                                    preferred_element_type=f32)
            ob = jnp.sum(jnp.where(diag, o / l, 0.0), axis=0, keepdims=True)
            oh_scr[...] = jnp.where(row == b, ob, oh_scr[...])

        @pl.when(step == B - 1)
        def _():
            with _scope("waitWo"):
                _wait_all(wo_buf, w_sems.at[2])

        @pl.when(b == B - 1)
        def _():
            off = pl.multiple_of(g * GD, GD)
            acc_scr[...] += jnp.dot(oh_scr[...].astype(bf16), wo_buf[pl.ds(off, GD), :],
                                    preferred_element_type=f32)

        return carry

    jax.lax.fori_loop(0, n_steps, step_body, 0)

    with _scope("e_ln"):
        hres = x32 + acc_scr[0:B, :]
        hn = _layernorm(hres)
        hn8 = _pad_rows(hn, 8).astype(bf16)
        r = jnp.sum(hn * wr_ref[...].astype(f32), axis=-1, keepdims=True)
        gate = jax.nn.sigmoid(r)
    with _scope("e_wgwait"):
        _wait_all(wg_buf, w_sems.at[3])
    with _scope("e_gate"):
        g = jnp.dot(hn8, wg_buf[...], preferred_element_type=f32)
        g = g * jax.nn.sigmoid(g)
    with _scope("e_wuwait"):
        _wait_all(wu_buf, w_sems.at[4])
    with _scope("e_up"):
        u = jnp.dot(hn8, wu_buf[...], preferred_element_type=f32)
        act = (g * u).astype(bf16)
    y = jnp.zeros((8, D), f32)
    for c in range(_WD_CHUNKS):
        rows = pl.ds(c * fc, fc)
        with _scope("e_wdwait"):
            _wait_all(wd_buf.at[rows], wd_sems.at[c])
        with _scope("e_down"):
            y = y + jnp.dot(act[:, c * fc:(c + 1) * fc], wd_buf[rows, :],
                            preferred_element_type=f32)
    with _scope("e_out"):
        out_buf[...] = (hres + (hn + y[0:B, :] * gate)).astype(out_buf.dtype)
        out_copy.start()
        out_copy.wait()


@jax.jit
def pallas_sequential_preLN__mha_block_cached__moe_arch_mod__decode_kernel(
    A_x: jax.Array,
    A_k_cache: jax.Array,
    A_v_cache: jax.Array,
    A_wq: jax.Array,
    A_wo: jax.Array,
    B_x: jax.Array,
    B_w_r: jax.Array,
    B_w_gate: jax.Array,
    B_w_up: jax.Array,
    B_w_down: jax.Array,
):
    B, Sq, D = A_x.shape
    _, H, S, Dh = A_k_cache.shape
    F = B_w_gate.shape[1]
    assert Sq == 1 and H % _HG == 0 and _HG <= 8 and B <= 8
    G = H // _HG
    GD = _HG * Dh
    x = A_x.reshape(B, D)
    kt = A_k_cache.transpose(0, 1, 3, 2).reshape(B, G, GD, S)
    vt = A_v_cache.transpose(0, 1, 3, 2).reshape(B, G, GD, S)
    wr = B_w_r.reshape(1, D)
    any_spec = pl.BlockSpec(memory_space=pl.ANY)
    vmem_spec = pl.BlockSpec(memory_space=pltpu.VMEM)
    bf16 = jnp.bfloat16
    out = pl.pallas_call(
        functools.partial(_kernel, B=B, G=G, S=S, Dh=Dh, D=D, F=F),
        out_shape=jax.ShapeDtypeStruct((B, D), A_x.dtype),
        in_specs=[any_spec, any_spec, any_spec, any_spec, any_spec, vmem_spec,
                  any_spec, any_spec, any_spec],
        out_specs=any_spec,
        scratch_shapes=[
            pltpu.VMEM((_NB, GD, S), bf16),
            pltpu.VMEM((B, D), bf16),
            pltpu.VMEM((D, H * Dh), bf16),
            pltpu.VMEM((H * Dh, D), bf16),
            pltpu.VMEM((D, F), bf16),
            pltpu.VMEM((D, F), bf16),
            pltpu.VMEM((F, D), bf16),
            pltpu.VMEM((G, 8, GD), jnp.float32),
            pltpu.VMEM((8, GD), jnp.float32),
            pltpu.VMEM((8, D), jnp.float32),
            pltpu.VMEM((B, D), bf16),
            pltpu.SemaphoreType.DMA((_NB,)),
            pltpu.SemaphoreType.DMA((6,)),
            pltpu.SemaphoreType.DMA((_WD_CHUNKS,)),
        ],
        compiler_params=pltpu.CompilerParams(vmem_limit_bytes=100 * 1024 * 1024,
                                             disable_bounds_checks=_NOBOUNDS),
    )(x, kt, vt, A_wq, A_wo, wr, B_w_gate, B_w_up, B_w_down)
    return out.reshape(B, Sq, D)
```

```python
import contextlib
import functools

import jax
import jax.numpy as jnp
import jax.experimental.pallas as pl
import jax.experimental.pallas.tpu as pltpu

_LN_EPS = 1e-5
_NB = 3
_HG = 2
_STRIP = 128
_WD_CHUNKS = 4
_WQ_RB = 320
_WO_WIN = (48, 640)
_WG_WIN = (320, 128)
_WD_WIN = (48, 640)
_COL_ORDER = (0, 1, 2, 3)
_KV_ROWS = (48, 336)
_SCOPES = False
_NOBOUNDS = True
_DBG_STEPS = None


def _scope(name):
    return jax.named_scope(name) if _SCOPES else contextlib.nullcontext()


def _layernorm(x):
    m = jnp.mean(x, axis=-1, keepdims=True)
    d = x - m
    v = jnp.mean(d * d, axis=-1, keepdims=True)
    return d / jnp.sqrt(v + _LN_EPS)


def _pad_rows(a, rows):
    return jnp.concatenate([a, jnp.zeros((rows - a.shape[0], a.shape[1]), a.dtype)], axis=0)


def _issue_windows(src, dst, sem, row_blocks, col_block):
    rows, cols = src.shape

    def start(r, nr, c, priority):
        win = (pl.ds(r, nr), pl.ds(c, col_block))
        pltpu.make_async_copy(src.at[win], dst.at[win], sem).start(priority=priority)

    if col_block == cols:
        row_block = row_blocks
        n = rows // row_block
        assert n % 4 == 0

        def body(i, carry):
            for u in range(4):
                r = pl.multiple_of((4 * i + u) * row_block, row_block)
                start(r, row_block, 0, u % 2)
            return carry

        jax.lax.fori_loop(0, n // 4, body, 0)
    else:
        if isinstance(row_blocks, int):
            row_blocks = (row_blocks,) * (rows // row_blocks)
        assert sum(row_blocks) == rows
        n = cols // col_block
        assert n % 4 == 0
        r = 0
        for nr in row_blocks:
            def body(i, carry, r=r, nr=nr):
                for u, cu in enumerate(_COL_ORDER):
                    c = pl.multiple_of((4 * i + cu) * col_block, col_block)
                    start(r, nr, c, u % 2)
                return carry

            jax.lax.fori_loop(0, n // 4, body, 0)
            r += nr


def _wait_all(dst, sem):
    pltpu.make_async_copy(dst, dst, sem).wait()


def _kernel(x_hbm, kt_hbm, vt_hbm, wq_hbm, wo_hbm, wr_hbm, wg_hbm, wu_hbm, wd_hbm,
            out_hbm,
            kv_buf, x_buf, wr_buf, wq_buf, wo_buf, wg_buf, wu_buf, wd_buf,
            q_scr, oh_scr, acc_scr, out_buf,
            kv_sems, w_sems, wd_sems,
            *, B, G, S, Dh, D, F):
    GD = _HG * Dh
    n_steps = _DBG_STEPS or B * G
    assert _NB == 3
    scale = Dh ** -0.5
    bf16 = jnp.bfloat16
    f32 = jnp.float32

    def slab_index(step):
        return step % B, step // B

    def issue_slab(src_hbm, step, slot):
        b, g = slab_index(step)
        _issue_windows(src_hbm.at[b, g], kv_buf.at[slot], kv_sems.at[slot], _KV_ROWS, _STRIP)

    def wait_slab(slot):
        _wait_all(kv_buf.at[slot], kv_sems.at[slot])

    x_copy = pltpu.make_async_copy(x_hbm, x_buf, w_sems.at[0])
    wr_copy = pltpu.make_async_copy(wr_hbm, wr_buf, w_sems.at[6])
    out_copy = pltpu.make_async_copy(out_buf, out_hbm, w_sems.at[5])
    fc = F // _WD_CHUNKS

    with _scope("p_issue"):
        x_copy.start()
        wr_copy.start()
        _issue_windows(wq_hbm, wq_buf, w_sems.at[1], _WQ_RB, _STRIP)
        issue_slab(kt_hbm, 0, 0)
        issue_slab(vt_hbm, 0, 1)

    with _scope("p_ln"):
        x_copy.wait()
        x32 = x_buf[...].astype(f32)
        xn = _pad_rows(_layernorm(x32), 8).astype(bf16)
    with _scope("p_wqwait"):
        _wait_all(wq_buf, w_sems.at[1])
    with _scope("p_qproj"):
        q_all = jnp.dot(xn, wq_buf[...], preferred_element_type=f32)
        for g in range(G):
            q_scr[g] = q_all[:, g * GD:(g + 1) * GD]
        acc_scr[...] = jnp.zeros_like(acc_scr)
        oh_scr[...] = jnp.zeros_like(oh_scr)

    row = jax.lax.broadcasted_iota(jnp.int32, (8, GD), 0)
    lane = jax.lax.broadcasted_iota(jnp.int32, (8, GD), 1)
    diag = jnp.logical_and(lane >= row * Dh, lane < (row + 1) * Dh)

    def step_body(step, carry):
        b, g = slab_index(step)
        kslot = (2 * step) % _NB
        vslot = (2 * step + 1) % _NB
        nslot = (2 * step + 2) % _NB
        last = step == n_steps - 1

        @pl.when(jnp.logical_not(last))
        def _():
            with _scope("issueK"):
                issue_slab(kt_hbm, step + 1, nslot)

        @pl.when(last)
        def _():
            with _scope("issueW"):
                _issue_windows(wg_hbm, wg_buf, w_sems.at[3], *_WG_WIN)
                _issue_windows(wu_hbm, wu_buf, w_sems.at[4], *_WG_WIN)
                for c in range(_WD_CHUNKS):
                    rows = pl.ds(c * fc, fc)
                    _issue_windows(wd_hbm.at[rows], wd_buf.at[rows], wd_sems.at[c], *_WD_WIN)

        qb = jnp.sum(jnp.where(row == b, q_scr[g], 0.0), axis=0, keepdims=True)
        q = jnp.where(diag, qb, 0.0).astype(bf16)
        with _scope("waitK"):
            wait_slab(kslot)
        with _scope("qk"):
            s = jnp.dot(q, kv_buf[kslot], preferred_element_type=f32)

        @pl.when(jnp.logical_not(last))
        def _():
            with _scope("issueV"):
                issue_slab(vt_hbm, step + 1, kslot)

        @pl.when(step == 0)
        def _():
            with _scope("issueWo"):
                _issue_windows(wo_hbm, wo_buf, w_sems.at[2], *_WO_WIN)

        m = jnp.max(s, axis=1, keepdims=True)
        p = jnp.exp((s - m) * scale)
        l = jnp.sum(p, axis=1, keepdims=True)
        with _scope("waitV"):
            wait_slab(vslot)
        with _scope("pv"):
            o = jax.lax.dot_general(p.astype(bf16), kv_buf[vslot], (((1,), (1,)), ((), ())),
                                    preferred_element_type=f32)
            ob = jnp.sum(jnp.where(diag, o / l, 0.0), axis=0, keepdims=True)
            oh_scr[...] = jnp.where(row == b, ob, oh_scr[...])

        @pl.when(step == B - 1)
        def _():
            with _scope("waitWo"):
                _wait_all(wo_buf, w_sems.at[2])

        @pl.when(b == B - 1)
        def _():
            off = pl.multiple_of(g * GD, GD)
            acc_scr[...] += jnp.dot(oh_scr[...].astype(bf16), wo_buf[pl.ds(off, GD), :],
                                    preferred_element_type=f32)

        return carry

    jax.lax.fori_loop(0, n_steps, step_body, 0)

    with _scope("e_ln"):
        hres = x32 + acc_scr[0:B, :]
        hn = _layernorm(hres)
        hn8 = _pad_rows(hn, 8).astype(bf16)
        wr_copy.wait()
        wr = wr_buf[...].astype(f32).reshape(1, D)
        r = jnp.sum(hn * wr, axis=-1, keepdims=True)
        gate = jax.nn.sigmoid(r)
    with _scope("e_wgwait"):
        _wait_all(wg_buf, w_sems.at[3])
    with _scope("e_gate"):
        g = jnp.dot(hn8, wg_buf[...], preferred_element_type=f32)
        g = g * jax.nn.sigmoid(g)
    with _scope("e_wuwait"):
        _wait_all(wu_buf, w_sems.at[4])
    with _scope("e_up"):
        u = jnp.dot(hn8, wu_buf[...], preferred_element_type=f32)
        act = (g * u).astype(bf16)
    y = jnp.zeros((8, D), f32)
    for c in range(_WD_CHUNKS):
        rows = pl.ds(c * fc, fc)
        with _scope("e_wdwait"):
            _wait_all(wd_buf.at[rows], wd_sems.at[c])
        with _scope("e_down"):
            y = y + jnp.dot(act[:, c * fc:(c + 1) * fc], wd_buf[rows, :],
                            preferred_element_type=f32)
    with _scope("e_out"):
        out_buf[...] = (hres + (hn + y[0:B, :] * gate)).astype(out_buf.dtype)
        out_copy.start()
        out_copy.wait()


@jax.jit
def pallas_sequential_preLN__mha_block_cached__moe_arch_mod__decode_kernel(
    A_x: jax.Array,
    A_k_cache: jax.Array,
    A_v_cache: jax.Array,
    A_wq: jax.Array,
    A_wo: jax.Array,
    B_x: jax.Array,
    B_w_r: jax.Array,
    B_w_gate: jax.Array,
    B_w_up: jax.Array,
    B_w_down: jax.Array,
):
    B, Sq, D = A_x.shape
    _, H, S, Dh = A_k_cache.shape
    F = B_w_gate.shape[1]
    assert Sq == 1 and H % _HG == 0 and _HG <= 8 and B <= 8
    G = H // _HG
    GD = _HG * Dh
    x = A_x.reshape(B, D)
    kt = A_k_cache.transpose(0, 1, 3, 2).reshape(B, G, GD, S)
    vt = A_v_cache.transpose(0, 1, 3, 2).reshape(B, G, GD, S)
    any_spec = pl.BlockSpec(memory_space=pl.ANY)
    bf16 = jnp.bfloat16
    out = pl.pallas_call(
        functools.partial(_kernel, B=B, G=G, S=S, Dh=Dh, D=D, F=F),
        out_shape=jax.ShapeDtypeStruct((B, D), A_x.dtype),
        in_specs=[any_spec] * 9,
        out_specs=any_spec,
        scratch_shapes=[
            pltpu.VMEM((_NB, GD, S), bf16),
            pltpu.VMEM((B, D), bf16),
            pltpu.VMEM((D,), bf16),
            pltpu.VMEM((D, H * Dh), bf16),
            pltpu.VMEM((H * Dh, D), bf16),
            pltpu.VMEM((D, F), bf16),
            pltpu.VMEM((D, F), bf16),
            pltpu.VMEM((F, D), bf16),
            pltpu.VMEM((G, 8, GD), jnp.float32),
            pltpu.VMEM((8, GD), jnp.float32),
            pltpu.VMEM((8, D), jnp.float32),
            pltpu.VMEM((B, D), bf16),
            pltpu.SemaphoreType.DMA((_NB,)),
            pltpu.SemaphoreType.DMA((7,)),
            pltpu.SemaphoreType.DMA((_WD_CHUNKS,)),
        ],
        compiler_params=pltpu.CompilerParams(vmem_limit_bytes=100 * 1024 * 1024,
                                             disable_bounds_checks=_NOBOUNDS),
    )(x, kt, vt, A_wq, A_wo, B_w_r, B_w_gate, B_w_up, B_w_down)
    return out.reshape(B, Sq, D)
```

```python
import functools

import jax
import jax.numpy as jnp
import jax.experimental.pallas as pl
import jax.experimental.pallas.tpu as pltpu

_LN_EPS = 1e-5
_NB = 3
_HG = 2
_STRIP = 128
_KV_ROWS = (48, 336)
_WQ_ROWS = 320
_ROW_WIN = 48
_WD_CHUNKS = 4


def _layernorm(x):
    m = jnp.mean(x, axis=-1, keepdims=True)
    d = x - m
    v = jnp.mean(d * d, axis=-1, keepdims=True)
    return d / jnp.sqrt(v + _LN_EPS)


def _pad_rows(a, rows):
    return jnp.concatenate([a, jnp.zeros((rows - a.shape[0], a.shape[1]), a.dtype)], axis=0)


def _start_window(src, dst, sem, win, priority):
    pltpu.make_async_copy(src.at[win], dst.at[win], sem).start(priority=priority)


def _issue_strips(src, dst, sem, heights):
    rows, cols = src.shape
    if isinstance(heights, int):
        heights = (heights,) * (rows // heights)
    assert sum(heights) == rows and cols % (4 * _STRIP) == 0
    r = 0
    for nr in heights:
        def body(i, carry, r=r, nr=nr):
            for u in range(4):
                c = pl.multiple_of((4 * i + u) * _STRIP, _STRIP)
                _start_window(src, dst, sem, (pl.ds(r, nr), pl.ds(c, _STRIP)), u % 2)
            return carry

        jax.lax.fori_loop(0, cols // (4 * _STRIP), body, 0)
        r += nr


def _issue_row_windows(src, dst, sem):
    rows, _ = src.shape
    assert rows % (4 * _ROW_WIN) == 0

    def body(i, carry):
        for u in range(4):
            r = pl.multiple_of((4 * i + u) * _ROW_WIN, _ROW_WIN)
            _start_window(src, dst, sem, (pl.ds(r, _ROW_WIN), slice(None)), u % 2)
        return carry

    jax.lax.fori_loop(0, rows // (4 * _ROW_WIN), body, 0)


def _wait_all(dst, sem):
    pltpu.make_async_copy(dst, dst, sem).wait()


def _kernel(x_hbm, kt_hbm, vt_hbm, wq_hbm, wo_hbm, wr_hbm, wg_hbm, wu_hbm, wd_hbm,
            out_hbm,
            kv_buf, x_buf, wr_buf, wq_buf, wo_buf, wg_buf, wu_buf, wd_buf,
            q_scr, oh_scr, acc_scr, out_buf,
            kv_sems, w_sems, wd_sems,
            *, B, G, Dh, D, F):
    GD = _HG * Dh
    n_steps = B * G
    scale = Dh ** -0.5
    bf16 = jnp.bfloat16
    f32 = jnp.float32

    def slab_index(step):
        return step % B, step // B

    def issue_slab(src_hbm, step, slot):
        b, g = slab_index(step)
        _issue_strips(src_hbm.at[b, g], kv_buf.at[slot], kv_sems.at[slot], _KV_ROWS)

    def wait_slab(slot):
        _wait_all(kv_buf.at[slot], kv_sems.at[slot])

    x_copy = pltpu.make_async_copy(x_hbm, x_buf, w_sems.at[0])
    wr_copy = pltpu.make_async_copy(wr_hbm, wr_buf, w_sems.at[1])
    out_copy = pltpu.make_async_copy(out_buf, out_hbm, w_sems.at[2])
    wq_sem, wo_sem, wg_sem, wu_sem = (w_sems.at[i] for i in range(3, 7))
    fc = F // _WD_CHUNKS
    wd_rows = [pl.ds(c * fc, fc) for c in range(_WD_CHUNKS)]

    x_copy.start()
    wr_copy.start()
    _issue_strips(wq_hbm, wq_buf, wq_sem, _WQ_ROWS)
    issue_slab(kt_hbm, 0, 0)
    issue_slab(vt_hbm, 0, 1)

    x_copy.wait()
    x32 = x_buf[...].astype(f32)
    xn = _pad_rows(_layernorm(x32), 8).astype(bf16)
    _wait_all(wq_buf, wq_sem)
    q_all = jnp.dot(xn, wq_buf[...], preferred_element_type=f32)
    for g in range(G):
        q_scr[g] = q_all[:, g * GD:(g + 1) * GD]
    acc_scr[...] = jnp.zeros_like(acc_scr)
    oh_scr[...] = jnp.zeros_like(oh_scr)

    row = jax.lax.broadcasted_iota(jnp.int32, (8, GD), 0)
    lane = jax.lax.broadcasted_iota(jnp.int32, (8, GD), 1)
    diag = jnp.logical_and(lane >= row * Dh, lane < (row + 1) * Dh)

    def step_body(step, carry):
        b, g = slab_index(step)
        kslot = (2 * step) % _NB
        vslot = (2 * step + 1) % _NB
        nslot = (2 * step + 2) % _NB
        last = step == n_steps - 1

        @pl.when(jnp.logical_not(last))
        def _():
            issue_slab(kt_hbm, step + 1, nslot)

        @pl.when(last)
        def _():
            _issue_strips(wg_hbm, wg_buf, wg_sem, _WQ_ROWS)
            _issue_strips(wu_hbm, wu_buf, wu_sem, _WQ_ROWS)
            for c, rows in enumerate(wd_rows):
                _issue_row_windows(wd_hbm.at[rows], wd_buf.at[rows], wd_sems.at[c])

        qb = jnp.sum(jnp.where(row == b, q_scr[g], 0.0), axis=0, keepdims=True)
        q = jnp.where(diag, qb, 0.0).astype(bf16)
        wait_slab(kslot)
        s = jnp.dot(q, kv_buf[kslot], preferred_element_type=f32)

        @pl.when(jnp.logical_not(last))
        def _():
            issue_slab(vt_hbm, step + 1, kslot)

        @pl.when(step == 0)
        def _():
            _issue_row_windows(wo_hbm, wo_buf, wo_sem)

        m = jnp.max(s, axis=1, keepdims=True)
        p = jnp.exp((s - m) * scale)
        l = jnp.sum(p, axis=1, keepdims=True)
        wait_slab(vslot)
        o = jax.lax.dot_general(p.astype(bf16), kv_buf[vslot], (((1,), (1,)), ((), ())),
                                preferred_element_type=f32)
        ob = jnp.sum(jnp.where(diag, o / l, 0.0), axis=0, keepdims=True)
        oh_scr[...] = jnp.where(row == b, ob, oh_scr[...])

        @pl.when(step == B - 1)
        def _():
            _wait_all(wo_buf, wo_sem)

        @pl.when(b == B - 1)
        def _():
            off = pl.multiple_of(g * GD, GD)
            acc_scr[...] += jnp.dot(oh_scr[...].astype(bf16), wo_buf[pl.ds(off, GD), :],
                                    preferred_element_type=f32)

        return carry

    jax.lax.fori_loop(0, n_steps, step_body, 0)

    h = x32 + acc_scr[0:B, :]
    hn = _layernorm(h)
    hn8 = _pad_rows(hn, 8).astype(bf16)
    wr_copy.wait()
    wr = wr_buf[...].astype(f32).reshape(1, D)
    gate = jax.nn.sigmoid(jnp.sum(hn * wr, axis=-1, keepdims=True))
    _wait_all(wg_buf, wg_sem)
    gt = jnp.dot(hn8, wg_buf[...], preferred_element_type=f32)
    gt = gt * jax.nn.sigmoid(gt)
    _wait_all(wu_buf, wu_sem)
    up = jnp.dot(hn8, wu_buf[...], preferred_element_type=f32)
    act = (gt * up).astype(bf16)
    y = jnp.zeros((8, D), f32)
    for c, rows in enumerate(wd_rows):
        _wait_all(wd_buf.at[rows], wd_sems.at[c])
        y = y + jnp.dot(act[:, c * fc:(c + 1) * fc], wd_buf[rows, :],
                        preferred_element_type=f32)
    out_buf[...] = (h + (hn + y[0:B, :] * gate)).astype(out_buf.dtype)
    out_copy.start()
    out_copy.wait()


@jax.jit
def pallas_sequential_preLN__mha_block_cached__moe_arch_mod__decode_kernel(
    A_x: jax.Array,
    A_k_cache: jax.Array,
    A_v_cache: jax.Array,
    A_wq: jax.Array,
    A_wo: jax.Array,
    B_x: jax.Array,
    B_w_r: jax.Array,
    B_w_gate: jax.Array,
    B_w_up: jax.Array,
    B_w_down: jax.Array,
):
    del B_x
    B, Sq, D = A_x.shape
    _, H, S, Dh = A_k_cache.shape
    F = B_w_gate.shape[1]
    assert Sq == 1 and H % _HG == 0 and _HG <= 8 and B <= 8 and _NB == 3
    G = H // _HG
    GD = _HG * Dh
    x = A_x.reshape(B, D)
    kt = A_k_cache.transpose(0, 1, 3, 2).reshape(B, G, GD, S)
    vt = A_v_cache.transpose(0, 1, 3, 2).reshape(B, G, GD, S)
    bf16 = jnp.bfloat16
    out = pl.pallas_call(
        functools.partial(_kernel, B=B, G=G, Dh=Dh, D=D, F=F),
        out_shape=jax.ShapeDtypeStruct((B, D), A_x.dtype),
        in_specs=[pl.BlockSpec(memory_space=pl.ANY)] * 9,
        out_specs=pl.BlockSpec(memory_space=pl.ANY),
        scratch_shapes=[
            pltpu.VMEM((_NB, GD, S), bf16),
            pltpu.VMEM((B, D), bf16),
            pltpu.VMEM((D,), bf16),
            pltpu.VMEM((D, H * Dh), bf16),
            pltpu.VMEM((H * Dh, D), bf16),
            pltpu.VMEM((D, F), bf16),
            pltpu.VMEM((D, F), bf16),
            pltpu.VMEM((F, D), bf16),
            pltpu.VMEM((G, 8, GD), jnp.float32),
            pltpu.VMEM((8, GD), jnp.float32),
            pltpu.VMEM((8, D), jnp.float32),
            pltpu.VMEM((B, D), bf16),
            pltpu.SemaphoreType.DMA((_NB,)),
            pltpu.SemaphoreType.DMA((7,)),
            pltpu.SemaphoreType.DMA((_WD_CHUNKS,)),
        ],
        compiler_params=pltpu.CompilerParams(vmem_limit_bytes=64 * 1024 * 1024),
    )(x, kt, vt, A_wq, A_wo, B_w_r, B_w_gate, B_w_up, B_w_down)
    return out.reshape(B, Sq, D)
```

```python
import functools

import jax
import jax.numpy as jnp
import jax.experimental.pallas as pl
import jax.experimental.pallas.tpu as pltpu

_LN_EPS = 1e-5
_NB = 3
_HG = 2
_STRIP = 128
_K_PLAN = ((80, 0, 0), (304, 1, 16))
_V_PLAN = ((384, 0, 24),)
_WQ_PLAN = ((320, 0, 0), (320, 0, 0))
_ROW_WIN = 48
_WD_CHUNKS = 4


def _layernorm(x):
    m = jnp.mean(x, axis=-1, keepdims=True)
    d = x - m
    v = jnp.mean(d * d, axis=-1, keepdims=True)
    return d / jnp.sqrt(v + _LN_EPS)


def _pad_rows(a, rows):
    return jnp.concatenate([a, jnp.zeros((rows - a.shape[0], a.shape[1]), a.dtype)], axis=0)


def _start_window(src, dst, sem, win, priority):
    pltpu.make_async_copy(src.at[win], dst.at[win], sem).start(priority=priority)


def _issue_strips(src, dst, sem, plan):
    rows, cols = src.shape
    n = cols // _STRIP
    assert sum(p[0] for p in plan) == rows and n % 4 == 0
    r = 0
    for height, flip, first in plan:
        assert first % 2 == 0

        def body(i, carry, r=r, height=height, flip=flip, first=first):
            for u in range(4):
                strip = 4 * i + u
                if first:
                    strip = (strip + first) % n
                c = pl.multiple_of(strip * _STRIP, _STRIP)
                _start_window(src, dst, sem, (pl.ds(r, height), pl.ds(c, _STRIP)),
                              (u + flip) % 2)
            return carry

        jax.lax.fori_loop(0, n // 4, body, 0)
        r += height


def _issue_row_windows(src, dst, sem):
    rows, _ = src.shape
    assert rows % (4 * _ROW_WIN) == 0

    def body(i, carry):
        for u in range(4):
            r = pl.multiple_of((4 * i + u) * _ROW_WIN, _ROW_WIN)
            _start_window(src, dst, sem, (pl.ds(r, _ROW_WIN), slice(None)), u % 2)
        return carry

    jax.lax.fori_loop(0, rows // (4 * _ROW_WIN), body, 0)


def _wait_all(dst, sem):
    pltpu.make_async_copy(dst, dst, sem).wait()


def _kernel(x_hbm, kt_hbm, vt_hbm, wq_hbm, wo_hbm, wr_hbm, wg_hbm, wu_hbm, wd_hbm,
            out_hbm,
            kv_buf, x_buf, wr_buf, wq_buf, wo_buf, wg_buf, wu_buf, wd_buf,
            q_scr, oh_scr, acc_scr, out_buf,
            kv_sems, w_sems, wd_sems,
            *, B, G, Dh, D, F):
    GD = _HG * Dh
    n_steps = B * G
    scale = Dh ** -0.5
    bf16 = jnp.bfloat16
    f32 = jnp.float32

    def slab_index(step):
        return step % B, step // B

    def issue_slab(src_hbm, plan, step, slot):
        b, g = slab_index(step)
        _issue_strips(src_hbm.at[b, g], kv_buf.at[slot], kv_sems.at[slot], plan)

    def wait_slab(slot):
        _wait_all(kv_buf.at[slot], kv_sems.at[slot])

    x_copy = pltpu.make_async_copy(x_hbm, x_buf, w_sems.at[0])
    wr_copy = pltpu.make_async_copy(wr_hbm, wr_buf, w_sems.at[1])
    out_copy = pltpu.make_async_copy(out_buf, out_hbm, w_sems.at[2])
    wq_sem, wo_sem, wg_sem, wu_sem = (w_sems.at[i] for i in range(3, 7))
    fc = F // _WD_CHUNKS
    wd_rows = [pl.ds(c * fc, fc) for c in range(_WD_CHUNKS)]

    x_copy.start()
    wr_copy.start()
    _issue_strips(wq_hbm, wq_buf, wq_sem, _WQ_PLAN)
    issue_slab(kt_hbm, _K_PLAN, 0, 0)
    issue_slab(vt_hbm, _V_PLAN, 0, 1)

    x_copy.wait()
    x32 = x_buf[...].astype(f32)
    xn = _pad_rows(_layernorm(x32), 8).astype(bf16)
    _wait_all(wq_buf, wq_sem)
    q_all = jnp.dot(xn, wq_buf[...], preferred_element_type=f32)
    for g in range(G):
        q_scr[g] = q_all[:, g * GD:(g + 1) * GD]
    acc_scr[...] = jnp.zeros_like(acc_scr)
    oh_scr[...] = jnp.zeros_like(oh_scr)

    row = jax.lax.broadcasted_iota(jnp.int32, (8, GD), 0)
    lane = jax.lax.broadcasted_iota(jnp.int32, (8, GD), 1)
    diag = jnp.logical_and(lane >= row * Dh, lane < (row + 1) * Dh)

    def step_body(step, carry):
        b, g = slab_index(step)
        kslot = (2 * step) % _NB
        vslot = (2 * step + 1) % _NB
        nslot = (2 * step + 2) % _NB
        last = step == n_steps - 1

        @pl.when(jnp.logical_not(last))
        def _():
            issue_slab(kt_hbm, _K_PLAN, step + 1, nslot)

        @pl.when(last)
        def _():
            _issue_strips(wg_hbm, wg_buf, wg_sem, _WQ_PLAN)
            _issue_strips(wu_hbm, wu_buf, wu_sem, _WQ_PLAN)
            for c, rows in enumerate(wd_rows):
                _issue_row_windows(wd_hbm.at[rows], wd_buf.at[rows], wd_sems.at[c])

        qb = jnp.sum(jnp.where(row == b, q_scr[g], 0.0), axis=0, keepdims=True)
        q = jnp.where(diag, qb, 0.0).astype(bf16)
        wait_slab(kslot)
        s = jnp.dot(q, kv_buf[kslot], preferred_element_type=f32)

        @pl.when(jnp.logical_not(last))
        def _():
            issue_slab(vt_hbm, _V_PLAN, step + 1, kslot)

        @pl.when(step == 0)
        def _():
            _issue_row_windows(wo_hbm, wo_buf, wo_sem)

        m = jnp.max(s, axis=1, keepdims=True)
        p = jnp.exp((s - m) * scale)
        l = jnp.sum(p, axis=1, keepdims=True)
        wait_slab(vslot)
        o = jax.lax.dot_general(p.astype(bf16), kv_buf[vslot], (((1,), (1,)), ((), ())),
                                preferred_element_type=f32)
        ob = jnp.sum(jnp.where(diag, o / l, 0.0), axis=0, keepdims=True)
        oh_scr[...] = jnp.where(row == b, ob, oh_scr[...])

        @pl.when(step == B - 1)
        def _():
            _wait_all(wo_buf, wo_sem)

        @pl.when(b == B - 1)
        def _():
            off = pl.multiple_of(g * GD, GD)
            acc_scr[...] += jnp.dot(oh_scr[...].astype(bf16), wo_buf[pl.ds(off, GD), :],
                                    preferred_element_type=f32)

        return carry

    jax.lax.fori_loop(0, n_steps, step_body, 0)

    h = x32 + acc_scr[0:B, :]
    hn = _layernorm(h)
    hn8 = _pad_rows(hn, 8).astype(bf16)
    wr_copy.wait()
    wr = wr_buf[...].astype(f32).reshape(1, D)
    gate = jax.nn.sigmoid(jnp.sum(hn * wr, axis=-1, keepdims=True))
    _wait_all(wg_buf, wg_sem)
    gt = jnp.dot(hn8, wg_buf[...], preferred_element_type=f32)
    gt = gt * jax.nn.sigmoid(gt)
    _wait_all(wu_buf, wu_sem)
    up = jnp.dot(hn8, wu_buf[...], preferred_element_type=f32)
    act = (gt * up).astype(bf16)
    y = jnp.zeros((8, D), f32)
    for c, rows in enumerate(wd_rows):
        _wait_all(wd_buf.at[rows], wd_sems.at[c])
        y = y + jnp.dot(act[:, c * fc:(c + 1) * fc], wd_buf[rows, :],
                        preferred_element_type=f32)
    out_buf[...] = (h + (hn + y[0:B, :] * gate)).astype(out_buf.dtype)
    out_copy.start()
    out_copy.wait()


@jax.jit
def pallas_sequential_preLN__mha_block_cached__moe_arch_mod__decode_kernel(
    A_x: jax.Array,
    A_k_cache: jax.Array,
    A_v_cache: jax.Array,
    A_wq: jax.Array,
    A_wo: jax.Array,
    B_x: jax.Array,
    B_w_r: jax.Array,
    B_w_gate: jax.Array,
    B_w_up: jax.Array,
    B_w_down: jax.Array,
):
    del B_x
    B, Sq, D = A_x.shape
    _, H, S, Dh = A_k_cache.shape
    F = B_w_gate.shape[1]
    assert Sq == 1 and H % _HG == 0 and _HG <= 8 and B <= 8 and _NB == 3
    G = H // _HG
    GD = _HG * Dh
    x = A_x.reshape(B, D)
    kt = A_k_cache.transpose(0, 1, 3, 2).reshape(B, G, GD, S)
    vt = A_v_cache.transpose(0, 1, 3, 2).reshape(B, G, GD, S)
    bf16 = jnp.bfloat16
    out = pl.pallas_call(
        functools.partial(_kernel, B=B, G=G, Dh=Dh, D=D, F=F),
        out_shape=jax.ShapeDtypeStruct((B, D), A_x.dtype),
        in_specs=[pl.BlockSpec(memory_space=pl.ANY)] * 9,
        out_specs=pl.BlockSpec(memory_space=pl.ANY),
        scratch_shapes=[
            pltpu.VMEM((_NB, GD, S), bf16),
            pltpu.VMEM((B, D), bf16),
            pltpu.VMEM((D,), bf16),
            pltpu.VMEM((D, H * Dh), bf16),
            pltpu.VMEM((H * Dh, D), bf16),
            pltpu.VMEM((D, F), bf16),
            pltpu.VMEM((D, F), bf16),
            pltpu.VMEM((F, D), bf16),
            pltpu.VMEM((G, 8, GD), jnp.float32),
            pltpu.VMEM((8, GD), jnp.float32),
            pltpu.VMEM((8, D), jnp.float32),
            pltpu.VMEM((B, D), bf16),
            pltpu.SemaphoreType.DMA((_NB,)),
            pltpu.SemaphoreType.DMA((7,)),
            pltpu.SemaphoreType.DMA((_WD_CHUNKS,)),
        ],
        compiler_params=pltpu.CompilerParams(vmem_limit_bytes=64 * 1024 * 1024),
    )(x, kt, vt, A_wq, A_wo, B_w_r, B_w_gate, B_w_up, B_w_down)
    return out.reshape(B, Sq, D)
```

```python
import functools

import jax
import jax.numpy as jnp
import jax.experimental.pallas as pl
import jax.experimental.pallas.tpu as pltpu

_LN_EPS = 1e-5
_NB = 3
_HG = 2
_STRIP = 128
_K_PLAN = ((48, 336), (((0, 0, 18), (1, 1, 23)), ((0, 1, 28), (1, 0, 20))))
_V_PLAN = ((384,), (((0, 0, 24), (0, 1, 12)),))
_WQ_PLAN = ((320, 320), (((0, 0, 0), (0, 1, 0)), ((1, 0, 0), (1, 1, 0))))
_ROW_WIN = 48
_WD_CHUNKS = 4


def _layernorm(x):
    m = jnp.mean(x, axis=-1, keepdims=True)
    d = x - m
    v = jnp.mean(d * d, axis=-1, keepdims=True)
    return d / jnp.sqrt(v + _LN_EPS)


def _pad_rows(a, rows):
    return jnp.concatenate([a, jnp.zeros((rows - a.shape[0], a.shape[1]), a.dtype)], axis=0)


def _start_window(src, dst, sem, win, priority):
    pltpu.make_async_copy(src.at[win], dst.at[win], sem).start(priority=priority)


def _issue_strips(src, dst, sem, plan):
    heights, phases = plan
    rows, cols = src.shape
    pairs = cols // (2 * _STRIP)
    assert sum(heights) == rows and cols % (4 * _STRIP) == 0
    assert sorted(lane[:2] for phase in phases for lane in phase) == sorted(
        (part, parity) for part in range(len(heights)) for parity in range(2))
    for phase in phases:
        def body(i, carry, phase=phase):
            for u in range(2):
                for queue, (part, parity, first) in enumerate(phase):
                    pair = (2 * i + u + first) % pairs if first else 2 * i + u
                    c = pl.multiple_of((2 * pair + parity) * _STRIP, _STRIP)
                    win = (pl.ds(sum(heights[:part]), heights[part]), pl.ds(c, _STRIP))
                    _start_window(src, dst, sem, win, queue)
            return carry

        jax.lax.fori_loop(0, pairs // 2, body, 0)


def _issue_row_windows(src, dst, sem):
    rows, _ = src.shape
    assert rows % (4 * _ROW_WIN) == 0

    def body(i, carry):
        for u in range(4):
            r = pl.multiple_of((4 * i + u) * _ROW_WIN, _ROW_WIN)
            _start_window(src, dst, sem, (pl.ds(r, _ROW_WIN), slice(None)), u % 2)
        return carry

    jax.lax.fori_loop(0, rows // (4 * _ROW_WIN), body, 0)


def _wait_all(dst, sem):
    pltpu.make_async_copy(dst, dst, sem).wait()


def _kernel(x_hbm, kt_hbm, vt_hbm, wq_hbm, wo_hbm, wr_hbm, wg_hbm, wu_hbm, wd_hbm,
            out_hbm,
            kv_buf, x_buf, wr_buf, wq_buf, wo_buf, wg_buf, wu_buf, wd_buf,
            q_scr, oh_scr, acc_scr, out_buf,
            kv_sems, w_sems, wd_sems,
            *, B, G, Dh, D, F):
    GD = _HG * Dh
    n_steps = B * G
    scale = Dh ** -0.5
    bf16 = jnp.bfloat16
    f32 = jnp.float32

    def slab_index(step):
        return step % B, step // B

    def issue_slab(src_hbm, plan, step, slot):
        b, g = slab_index(step)
        _issue_strips(src_hbm.at[b, g], kv_buf.at[slot], kv_sems.at[slot], plan)

    def wait_slab(slot):
        _wait_all(kv_buf.at[slot], kv_sems.at[slot])

    x_copy = pltpu.make_async_copy(x_hbm, x_buf, w_sems.at[0])
    wr_copy = pltpu.make_async_copy(wr_hbm, wr_buf, w_sems.at[1])
    out_copy = pltpu.make_async_copy(out_buf, out_hbm, w_sems.at[2])
    wq_sem, wo_sem, wg_sem, wu_sem = (w_sems.at[i] for i in range(3, 7))
    fc = F // _WD_CHUNKS
    wd_rows = [pl.ds(c * fc, fc) for c in range(_WD_CHUNKS)]

    x_copy.start()
    wr_copy.start()
    _issue_strips(wq_hbm, wq_buf, wq_sem, _WQ_PLAN)
    issue_slab(kt_hbm, _K_PLAN, 0, 0)
    issue_slab(vt_hbm, _V_PLAN, 0, 1)

    x_copy.wait()
    x32 = x_buf[...].astype(f32)
    xn = _pad_rows(_layernorm(x32), 8).astype(bf16)
    _wait_all(wq_buf, wq_sem)
    q_all = jnp.dot(xn, wq_buf[...], preferred_element_type=f32)
    for g in range(G):
        q_scr[g] = q_all[:, g * GD:(g + 1) * GD]
    acc_scr[...] = jnp.zeros_like(acc_scr)
    oh_scr[...] = jnp.zeros_like(oh_scr)

    row = jax.lax.broadcasted_iota(jnp.int32, (8, GD), 0)
    lane = jax.lax.broadcasted_iota(jnp.int32, (8, GD), 1)
    diag = jnp.logical_and(lane >= row * Dh, lane < (row + 1) * Dh)

    def step_body(step, carry):
        b, g = slab_index(step)
        kslot = (2 * step) % _NB
        vslot = (2 * step + 1) % _NB
        nslot = (2 * step + 2) % _NB
        last = step == n_steps - 1

        @pl.when(jnp.logical_not(last))
        def _():
            issue_slab(kt_hbm, _K_PLAN, step + 1, nslot)

        @pl.when(last)
        def _():
            _issue_strips(wg_hbm, wg_buf, wg_sem, _WQ_PLAN)
            _issue_strips(wu_hbm, wu_buf, wu_sem, _WQ_PLAN)
            for c, rows in enumerate(wd_rows):
                _issue_row_windows(wd_hbm.at[rows], wd_buf.at[rows], wd_sems.at[c])

        qb = jnp.sum(jnp.where(row == b, q_scr[g], 0.0), axis=0, keepdims=True)
        q = jnp.where(diag, qb, 0.0).astype(bf16)
        wait_slab(kslot)
        s = jnp.dot(q, kv_buf[kslot], preferred_element_type=f32)

        @pl.when(jnp.logical_not(last))
        def _():
            issue_slab(vt_hbm, _V_PLAN, step + 1, kslot)

        @pl.when(step == 0)
        def _():
            _issue_row_windows(wo_hbm, wo_buf, wo_sem)

        m = jnp.max(s, axis=1, keepdims=True)
        p = jnp.exp((s - m) * scale)
        l = jnp.sum(p, axis=1, keepdims=True)
        wait_slab(vslot)
        o = jax.lax.dot_general(p.astype(bf16), kv_buf[vslot], (((1,), (1,)), ((), ())),
                                preferred_element_type=f32)
        ob = jnp.sum(jnp.where(diag, o / l, 0.0), axis=0, keepdims=True)
        oh_scr[...] = jnp.where(row == b, ob, oh_scr[...])

        @pl.when(step == B - 1)
        def _():
            _wait_all(wo_buf, wo_sem)

        @pl.when(b == B - 1)
        def _():
            off = pl.multiple_of(g * GD, GD)
            acc_scr[...] += jnp.dot(oh_scr[...].astype(bf16), wo_buf[pl.ds(off, GD), :],
                                    preferred_element_type=f32)

        return carry

    jax.lax.fori_loop(0, n_steps, step_body, 0)

    h = x32 + acc_scr[0:B, :]
    hn = _layernorm(h)
    hn8 = _pad_rows(hn, 8).astype(bf16)
    wr_copy.wait()
    wr = wr_buf[...].astype(f32).reshape(1, D)
    gate = jax.nn.sigmoid(jnp.sum(hn * wr, axis=-1, keepdims=True))
    _wait_all(wg_buf, wg_sem)
    gt = jnp.dot(hn8, wg_buf[...], preferred_element_type=f32)
    gt = gt * jax.nn.sigmoid(gt)
    _wait_all(wu_buf, wu_sem)
    up = jnp.dot(hn8, wu_buf[...], preferred_element_type=f32)
    act = (gt * up).astype(bf16)
    y = jnp.zeros((8, D), f32)
    for c, rows in enumerate(wd_rows):
        _wait_all(wd_buf.at[rows], wd_sems.at[c])
        y = y + jnp.dot(act[:, c * fc:(c + 1) * fc], wd_buf[rows, :],
                        preferred_element_type=f32)
    out_buf[...] = (h + (hn + y[0:B, :] * gate)).astype(out_buf.dtype)
    out_copy.start()
    out_copy.wait()


@jax.jit
def pallas_sequential_preLN__mha_block_cached__moe_arch_mod__decode_kernel(
    A_x: jax.Array,
    A_k_cache: jax.Array,
    A_v_cache: jax.Array,
    A_wq: jax.Array,
    A_wo: jax.Array,
    B_x: jax.Array,
    B_w_r: jax.Array,
    B_w_gate: jax.Array,
    B_w_up: jax.Array,
    B_w_down: jax.Array,
):
    del B_x
    B, Sq, D = A_x.shape
    _, H, S, Dh = A_k_cache.shape
    F = B_w_gate.shape[1]
    assert Sq == 1 and H % _HG == 0 and _HG <= 8 and B <= 8 and _NB == 3
    G = H // _HG
    GD = _HG * Dh
    x = A_x.reshape(B, D)
    kt = A_k_cache.transpose(0, 1, 3, 2).reshape(B, G, GD, S)
    vt = A_v_cache.transpose(0, 1, 3, 2).reshape(B, G, GD, S)
    bf16 = jnp.bfloat16
    out = pl.pallas_call(
        functools.partial(_kernel, B=B, G=G, Dh=Dh, D=D, F=F),
        out_shape=jax.ShapeDtypeStruct((B, D), A_x.dtype),
        in_specs=[pl.BlockSpec(memory_space=pl.ANY)] * 9,
        out_specs=pl.BlockSpec(memory_space=pl.ANY),
        scratch_shapes=[
            pltpu.VMEM((_NB, GD, S), bf16),
            pltpu.VMEM((B, D), bf16),
            pltpu.VMEM((D,), bf16),
            pltpu.VMEM((D, H * Dh), bf16),
            pltpu.VMEM((H * Dh, D), bf16),
            pltpu.VMEM((D, F), bf16),
            pltpu.VMEM((D, F), bf16),
            pltpu.VMEM((F, D), bf16),
            pltpu.VMEM((G, 8, GD), jnp.float32),
            pltpu.VMEM((8, GD), jnp.float32),
            pltpu.VMEM((8, D), jnp.float32),
            pltpu.VMEM((B, D), bf16),
            pltpu.SemaphoreType.DMA((_NB,)),
            pltpu.SemaphoreType.DMA((7,)),
            pltpu.SemaphoreType.DMA((_WD_CHUNKS,)),
        ],
        compiler_params=pltpu.CompilerParams(vmem_limit_bytes=64 * 1024 * 1024),
    )(x, kt, vt, A_wq, A_wo, B_w_r, B_w_gate, B_w_up, B_w_down)
    return out.reshape(B, Sq, D)
```

```python
import functools

import jax
import jax.numpy as jnp
import jax.experimental.pallas as pl
import jax.experimental.pallas.tpu as pltpu

_LN_EPS = 1e-5
_NB = 3
_HG = 2
_STRIP = 128
_K_PLAN = ((48, 336), (((0, 0, 16), (1, 1, 21)), ((0, 1, 26), (1, 0, 20))))
_V_PLAN = ((384,), (((0, 0, 24), (0, 1, 9)),))
_WQ_PLAN = ((320, 320), (((0, 0, 0), (0, 1, 0)), ((1, 0, 0), (1, 1, 0))))
_ROW_WIN = 48
_WD_CHUNKS = 4


def _layernorm(x):
    m = jnp.mean(x, axis=-1, keepdims=True)
    d = x - m
    v = jnp.mean(d * d, axis=-1, keepdims=True)
    return d / jnp.sqrt(v + _LN_EPS)


def _pad_rows(a, rows):
    return jnp.concatenate([a, jnp.zeros((rows - a.shape[0], a.shape[1]), a.dtype)], axis=0)


def _start_window(src, dst, sem, win, priority):
    pltpu.make_async_copy(src.at[win], dst.at[win], sem).start(priority=priority)


def _issue_strips(src, dst, sem, plan):
    heights, phases = plan
    rows, cols = src.shape
    pairs = cols // (2 * _STRIP)
    assert sum(heights) == rows and cols % (4 * _STRIP) == 0
    assert sorted(lane[:2] for phase in phases for lane in phase) == sorted(
        (part, parity) for part in range(len(heights)) for parity in range(2))
    for phase in phases:
        def body(i, carry, phase=phase):
            for u in range(2):
                for queue, (part, parity, first) in enumerate(phase):
                    pair = (2 * i + u + first) % pairs if first else 2 * i + u
                    c = pl.multiple_of((2 * pair + parity) * _STRIP, _STRIP)
                    win = (pl.ds(sum(heights[:part]), heights[part]), pl.ds(c, _STRIP))
                    _start_window(src, dst, sem, win, queue)
            return carry

        jax.lax.fori_loop(0, pairs // 2, body, 0)


def _issue_row_windows(src, dst, sem):
    rows, _ = src.shape
    assert rows % (4 * _ROW_WIN) == 0

    def body(i, carry):
        for u in range(4):
            r = pl.multiple_of((4 * i + u) * _ROW_WIN, _ROW_WIN)
            _start_window(src, dst, sem, (pl.ds(r, _ROW_WIN), slice(None)), u % 2)
        return carry

    jax.lax.fori_loop(0, rows // (4 * _ROW_WIN), body, 0)


def _wait_all(dst, sem):
    pltpu.make_async_copy(dst, dst, sem).wait()


def _kernel(x_hbm, kt_hbm, vt_hbm, wq_hbm, wo_hbm, wr_hbm, wg_hbm, wu_hbm, wd_hbm,
            out_hbm,
            kv_buf, x_buf, wr_buf, wq_buf, wo_buf, wg_buf, wu_buf, wd_buf,
            q_scr, oh_scr, acc_scr, out_buf,
            kv_sems, w_sems, wd_sems,
            *, B, G, Dh, D, F):
    GD = _HG * Dh
    n_steps = B * G
    scale = Dh ** -0.5
    bf16 = jnp.bfloat16
    f32 = jnp.float32

    def slab_index(step):
        return step % B, step // B

    def issue_slab(src_hbm, plan, step, slot):
        b, g = slab_index(step)
        _issue_strips(src_hbm.at[b, g], kv_buf.at[slot], kv_sems.at[slot], plan)

    def wait_slab(slot):
        _wait_all(kv_buf.at[slot], kv_sems.at[slot])

    x_copy = pltpu.make_async_copy(x_hbm, x_buf, w_sems.at[0])
    wr_copy = pltpu.make_async_copy(wr_hbm, wr_buf, w_sems.at[1])
    out_copy = pltpu.make_async_copy(out_buf, out_hbm, w_sems.at[2])
    wq_sem, wo_sem, wg_sem, wu_sem = (w_sems.at[i] for i in range(3, 7))
    fc = F // _WD_CHUNKS
    wd_rows = [pl.ds(c * fc, fc) for c in range(_WD_CHUNKS)]

    x_copy.start()
    wr_copy.start()
    _issue_strips(wq_hbm, wq_buf, wq_sem, _WQ_PLAN)
    issue_slab(kt_hbm, _K_PLAN, 0, 0)
    issue_slab(vt_hbm, _V_PLAN, 0, 1)

    x_copy.wait()
    x32 = x_buf[...].astype(f32)
    xn = _pad_rows(_layernorm(x32), 8).astype(bf16)
    _wait_all(wq_buf, wq_sem)
    q_all = jnp.dot(xn, wq_buf[...], preferred_element_type=f32)
    for g in range(G):
        q_scr[g] = q_all[:, g * GD:(g + 1) * GD]
    acc_scr[...] = jnp.zeros_like(acc_scr)
    oh_scr[...] = jnp.zeros_like(oh_scr)

    row = jax.lax.broadcasted_iota(jnp.int32, (8, GD), 0)
    lane = jax.lax.broadcasted_iota(jnp.int32, (8, GD), 1)
    diag = jnp.logical_and(lane >= row * Dh, lane < (row + 1) * Dh)

    def step_body(step, carry):
        b, g = slab_index(step)
        kslot = (2 * step) % _NB
        vslot = (2 * step + 1) % _NB
        nslot = (2 * step + 2) % _NB
        last = step == n_steps - 1

        @pl.when(jnp.logical_not(last))
        def _():
            issue_slab(kt_hbm, _K_PLAN, step + 1, nslot)

        @pl.when(last)
        def _():
            _issue_strips(wg_hbm, wg_buf, wg_sem, _WQ_PLAN)
            _issue_strips(wu_hbm, wu_buf, wu_sem, _WQ_PLAN)
            for c, rows in enumerate(wd_rows):
                _issue_row_windows(wd_hbm.at[rows], wd_buf.at[rows], wd_sems.at[c])

        qb = jnp.sum(jnp.where(row == b, q_scr[g], 0.0), axis=0, keepdims=True)
        q = jnp.where(diag, qb, 0.0).astype(bf16)
        wait_slab(kslot)
        s = jnp.dot(q, kv_buf[kslot], preferred_element_type=f32)

        @pl.when(jnp.logical_not(last))
        def _():
            issue_slab(vt_hbm, _V_PLAN, step + 1, kslot)

        wo_rows = pl.ds(pl.multiple_of(g * GD, GD), GD)

        @pl.when(b == 0)
        def _():
            _issue_row_windows(wo_hbm.at[wo_rows], wo_buf.at[wo_rows], wo_sem)

        m = jnp.max(s, axis=1, keepdims=True)
        p = jnp.exp((s - m) * scale)
        l = jnp.sum(p, axis=1, keepdims=True)
        wait_slab(vslot)
        o = jax.lax.dot_general(p.astype(bf16), kv_buf[vslot], (((1,), (1,)), ((), ())),
                                preferred_element_type=f32)
        ob = jnp.sum(jnp.where(diag, o / l, 0.0), axis=0, keepdims=True)
        oh_scr[...] = jnp.where(row == b, ob, oh_scr[...])

        @pl.when(b == B - 1)
        def _():
            _wait_all(wo_buf.at[wo_rows], wo_sem)
            acc_scr[...] += jnp.dot(oh_scr[...].astype(bf16), wo_buf[wo_rows, :],
                                    preferred_element_type=f32)

        return carry

    jax.lax.fori_loop(0, n_steps, step_body, 0)

    h = x32 + acc_scr[0:B, :]
    hn = _layernorm(h)
    hn8 = _pad_rows(hn, 8).astype(bf16)
    wr_copy.wait()
    wr = wr_buf[...].astype(f32).reshape(1, D)
    gate = jax.nn.sigmoid(jnp.sum(hn * wr, axis=-1, keepdims=True))
    _wait_all(wg_buf, wg_sem)
    gt = jnp.dot(hn8, wg_buf[...], preferred_element_type=f32)
    gt = gt * jax.nn.sigmoid(gt)
    _wait_all(wu_buf, wu_sem)
    up = jnp.dot(hn8, wu_buf[...], preferred_element_type=f32)
    act = (gt * up).astype(bf16)
    y = jnp.zeros((8, D), f32)
    for c, rows in enumerate(wd_rows):
        _wait_all(wd_buf.at[rows], wd_sems.at[c])
        y = y + jnp.dot(act[:, c * fc:(c + 1) * fc], wd_buf[rows, :],
                        preferred_element_type=f32)
    out_buf[...] = (h + (hn + y[0:B, :] * gate)).astype(out_buf.dtype)
    out_copy.start()
    out_copy.wait()


@jax.jit
def pallas_sequential_preLN__mha_block_cached__moe_arch_mod__decode_kernel(
    A_x: jax.Array,
    A_k_cache: jax.Array,
    A_v_cache: jax.Array,
    A_wq: jax.Array,
    A_wo: jax.Array,
    B_x: jax.Array,
    B_w_r: jax.Array,
    B_w_gate: jax.Array,
    B_w_up: jax.Array,
    B_w_down: jax.Array,
):
    del B_x
    B, Sq, D = A_x.shape
    _, H, S, Dh = A_k_cache.shape
    F = B_w_gate.shape[1]
    assert Sq == 1 and H % _HG == 0 and _HG <= 8 and 2 <= B <= 8 and _NB == 3
    G = H // _HG
    GD = _HG * Dh
    x = A_x.reshape(B, D)
    kt = A_k_cache.transpose(0, 1, 3, 2).reshape(B, G, GD, S)
    vt = A_v_cache.transpose(0, 1, 3, 2).reshape(B, G, GD, S)
    bf16 = jnp.bfloat16
    out = pl.pallas_call(
        functools.partial(_kernel, B=B, G=G, Dh=Dh, D=D, F=F),
        out_shape=jax.ShapeDtypeStruct((B, D), A_x.dtype),
        in_specs=[pl.BlockSpec(memory_space=pl.ANY)] * 9,
        out_specs=pl.BlockSpec(memory_space=pl.ANY),
        scratch_shapes=[
            pltpu.VMEM((_NB, GD, S), bf16),
            pltpu.VMEM((B, D), bf16),
            pltpu.VMEM((D,), bf16),
            pltpu.VMEM((D, H * Dh), bf16),
            pltpu.VMEM((H * Dh, D), bf16),
            pltpu.VMEM((D, F), bf16),
            pltpu.VMEM((D, F), bf16),
            pltpu.VMEM((F, D), bf16),
            pltpu.VMEM((G, 8, GD), jnp.float32),
            pltpu.VMEM((8, GD), jnp.float32),
            pltpu.VMEM((8, D), jnp.float32),
            pltpu.VMEM((B, D), bf16),
            pltpu.SemaphoreType.DMA((_NB,)),
            pltpu.SemaphoreType.DMA((7,)),
            pltpu.SemaphoreType.DMA((_WD_CHUNKS,)),
        ],
        compiler_params=pltpu.CompilerParams(vmem_limit_bytes=64 * 1024 * 1024),
    )(x, kt, vt, A_wq, A_wo, B_w_r, B_w_gate, B_w_up, B_w_down)
    return out.reshape(B, Sq, D)
```
